```python
import os as _os
_os.environ.setdefault("JAX_PLATFORMS", "cpu")
import jax
import jax.numpy as jnp

def _softmax(x, axis=-1):
    return jax.nn.softmax(x, axis=axis)
def _gelu(x):
    return jax.nn.gelu(x, approximate=True)
def _silu(x):
    return jax.nn.silu(x)
def _sigmoid(x):
    return jax.nn.sigmoid(x)
def _layernorm(x, axis=-1, eps=1e-5):
    m = jnp.mean(x, axis=axis, keepdims=True)
    v = jnp.var(x, axis=axis, keepdims=True)
    return (x - m) / jnp.sqrt(v + eps)
def _scatter_add(tgt, idx, src, axis=0):
    return tgt.at[idx].add(src)
def _segment_sum(src, seg, n):
    return jax.ops.segment_sum(src, seg, n)
class _Rng:
    def __init__(self, key):
        self._k = key
    def _next(self):
        self._k, sub = jax.random.split(self._k)
        return sub
    def normal(self, shape):
        return jax.random.normal(self._next(), shape, dtype=jnp.bfloat16)
    def randint(self, lo, hi, shape):
        return jax.random.randint(self._next(), shape, lo, hi, dtype=jnp.int32)
    def uniform(self, shape, lo=0.0, hi=1.0):
        return jax.random.uniform(self._next(), shape, jnp.bfloat16, lo, hi)
    def permutation(self, n):
        return jax.random.permutation(self._next(), n)


kernel_name = 'interleave_layers__linear_kernel_hedgehog__dense_activation_silu__prompt'

def setup_inputs():
    _rng = _Rng(jax.random.key(int.from_bytes(__import__("os").urandom(4), "little")))
    _w = (lambda a: (lambda t: t.astype(jnp.bfloat16) if jnp.issubdtype(t.dtype, jnp.floating) else t)(jnp.asarray(a)))
    def _A_setup():
        B, S, D, H = 1, 2048, 640, 32
        Dh = D // H
        return {
            "x": _w((lambda *s: _rng.normal(s) * 0.05)(B, S, D)),
            "wqkv": _w((lambda *s: _rng.normal(s) * 0.4)(D, 3 * D)),
            "w_phi": _w((lambda *s: _rng.normal(s) * 0.4)(H, Dh, Dh) * (Dh ** -0.5)),
            "wo": _w((lambda *s: _rng.normal(s) * 0.05)(D, D)),
        }
    _A_in = _A_setup()

    def _B_setup():
        B, S, D, F = 1, 2048, 640, 1728
        return {
            "x": _w((lambda *s: _rng.normal(s) * 0.05)(B, S, D)),
            "w1": _w((lambda *s: _rng.normal(s) * 1.6)(D, F) * (D ** -0.5)),
            "w2": _w((lambda *s: _rng.normal(s) * 1.6)(F, D) * (F ** -0.5)),
        }
    _B_in = _B_setup()

    return {
        "A_x": _A_in["x"],
        "A_wqkv": _A_in["wqkv"],
        "A_w_phi": _A_in["w_phi"],
        "A_wo": _A_in["wo"],
        "B_x": _B_in["x"],
        "B_w1": _B_in["w1"],
        "B_w2": _B_in["w2"],
    }

def reference(A_x, A_wqkv, A_w_phi, A_wo, B_x, B_w1, B_w2):
    def _A_ref(x, wqkv, w_phi, wo):
        B, S, D = x.shape
        H = 32; Dh = D // H
        qkv = (lambda x, *d: x.transpose(*d))((x @ wqkv).reshape(B, S, 3, H, Dh), 2, 0, 3, 1, 4)
        q, k, v = qkv[0], qkv[1], qkv[2]
        pq = jnp.einsum("bhsd,hdf->bhsf", q, w_phi)
        pk = jnp.einsum("bhsd,hdf->bhsf", k, w_phi)
        phi_q = jnp.concatenate([_softmax(pq, axis=-1), _softmax(-pq, axis=-1)], axis=-1)
        phi_k = jnp.concatenate([_softmax(pk, axis=-1), _softmax(-pk, axis=-1)], axis=-1)
        kv = jnp.einsum("bhsf,bhsd->bhfd", phi_k, v)
        z  = jnp.einsum("bhsf->bhf", phi_k)
        num = jnp.einsum("bhqf,bhfd->bhqd", phi_q, kv)
        den = jnp.einsum("bhqf,bhf->bhq", phi_q, z)[..., None] + 1e-6
        o = num / den
        return (lambda x, *d: x.transpose(*d))(o, 0, 2, 1, 3).reshape(B, S, D) @ wo

    def _B_ref(x, w1, w2):
        h = jnp.einsum("bsd,df->bsf", x, w1)
        h = _silu(h)
        out = jnp.einsum("bsf,fd->bsd", h, w2)
        return out

    x = A_x
    x = x + _A_ref(_layernorm(x, axis=-1), A_wqkv, A_w_phi, A_wo)
    x = x + _B_ref(_layernorm(x, axis=-1), B_w1, B_w2)
    x = x + _A_ref(_layernorm(x, axis=-1), A_wqkv, A_w_phi, A_wo)
    x = x + _B_ref(_layernorm(x, axis=-1), B_w1, B_w2)
    return x
```

```python
import jax
import jax.numpy as jnp
import jax.experimental.pallas as pl
import jax.experimental.pallas.tpu as pltpu

S = 2048
D = 640
H = 32
DH = D // H
F = 1728
G = 4
HG = H // G
GR = HG * DH
TB = 512
NB = S // TB
LN_EPS = 1e-5
DEN_EPS = 1e-6

_NT = (((1,), (1,)), ((), ()))

_PHI_LO = tuple(128 * ((2 * GR * g) // 128) for g in range(G))
_PHI_W = 384
_QK_LO = tuple(128 * ((GR * g) // 128) for g in range(G))
_QK_W = 256


def _layernorm_bf16(x):
    m = jnp.mean(x, axis=-1, keepdims=True)
    xc = x - m
    v = jnp.mean(xc * xc, axis=-1, keepdims=True)
    return (xc * jax.lax.rsqrt(v + LN_EPS)).astype(jnp.bfloat16)


def _dual_softmax_parts(pT):
    p4 = pT.reshape(G, DH, HG, TB)
    mx = jnp.max(p4, axis=1, keepdims=True)
    mn = jnp.min(p4, axis=1, keepdims=True)
    e1 = jnp.exp(p4 - mx)
    e2 = jnp.exp(mn - p4)
    s1 = jnp.sum(e1, axis=1, keepdims=True)
    s2 = jnp.sum(e2, axis=1, keepdims=True)
    return e1, e2, s1, s2


def _interleave_signs(f1, f2):
    return jnp.stack([f1, f2], axis=1).reshape(2 * D, TB)


def _kernel(x_ref, wphi_ref, wqkv_hbm, wo_hbm, w1_hbm, w2_hbm, o_ref,
            wqkv_v, wo_v, w1_v, w2_v, wT, x_scr, pq_scr, kvt, kvtm, zacc, zb_scr, sems):
    phase = pl.program_id(0)
    i = pl.program_id(1)
    row0 = pl.multiple_of(i * TB, TB)
    rows = pl.ds(row0, TB)

    def weight_copy(k):
        src, dst = ((wqkv_hbm, wqkv_v), (wo_hbm, wo_v), (w1_hbm, w1_v), (w2_hbm, w2_v))[k]
        return pltpu.make_async_copy(src, dst, sems.at[k])

    @pl.when(jnp.logical_and(phase == 0, i == 0))
    def _prologue():
        for k in range(4):
            weight_copy(k).start()
        rr = jax.lax.broadcasted_iota(jnp.int32, (D, DH), 0)
        cc = jax.lax.broadcasted_iota(jnp.int32, (D, DH), 1)
        rep = (((rr % GR) // HG) == cc).astype(jnp.bfloat16)
        bd_u = jax.lax.dot_general(rep, wphi_ref[...], _NT, preferred_element_type=jnp.float32)
        r2 = jax.lax.broadcasted_iota(jnp.int32, (D, D), 0)
        c2 = jax.lax.broadcasted_iota(jnp.int32, (D, D), 1)
        same_head = (c2 // DH) == (HG * (r2 // GR) + r2 % HG)
        bdp = jnp.where(same_head, bd_u, 0.0).astype(jnp.bfloat16)
        weight_copy(0).wait()
        for g in range(G):
            lo = _QK_LO[g]
            bd_g = bdp[GR * g:GR * (g + 1), lo:lo + _QK_W]
            for part in range(2):
                w_g = wqkv_v[:, part * D + lo:part * D + lo + _QK_W]
                wT[part * D + GR * g:part * D + GR * (g + 1), :] = jax.lax.dot_general(
                    bd_g, w_g, _NT, preferred_element_type=jnp.float32).astype(jnp.bfloat16)
        wT[2 * D:3 * D, :] = wqkv_v[:, 2 * D:3 * D].astype(jnp.float32).T.astype(jnp.bfloat16)

    @pl.when(jnp.logical_and(phase == 1, i == 0))
    def _wait_weights():
        for k in range(1, 4):
            weight_copy(k).wait()

    @pl.when(jnp.logical_and(phase > 0, i == 0))
    def _finalize_kv():
        r2 = jax.lax.broadcasted_iota(jnp.int32, (D, 2 * D), 0)
        c2 = jax.lax.broadcasted_iota(jnp.int32, (D, 2 * D), 1)
        same_head = (r2 // DH) == (HG * (c2 // (2 * GR)) + c2 % HG)
        kvtm[...] = jnp.where(same_head, kvt[...], 0.0).astype(jnp.bfloat16)
        z = jnp.sum(zacc[...], axis=1, keepdims=True)
        zb_scr[...] = jnp.broadcast_to(z, (2 * D, TB))

    @pl.when(jnp.logical_and(phase < 2, i == 0))
    def _zero_acc():
        kvt[...] = jnp.zeros_like(kvt)
        zacc[...] = jnp.zeros_like(zacc)

    @pl.when(phase > 0)
    def _part_b():
        e1, e2, s1, s2 = _dual_softmax_parts(pq_scr[:, rows])
        zb = zb_scr[...].reshape(G, 2, DH, HG, TB)
        d1 = jnp.sum(e1 * zb[:, 0], axis=1, keepdims=True)
        d2 = jnp.sum(e2 * zb[:, 1], axis=1, keepdims=True)
        r1 = 1.0 / s1
        r2 = 1.0 / s2
        den = d1 * r1 + d2 * r2 + DEN_EPS
        rden = 1.0 / den
        phi = _interleave_signs(e1 * (r1 * rden), e2 * (r2 * rden)).astype(jnp.bfloat16)
        pieces = []
        for g in range(G):
            lo = _PHI_LO[g]
            pieces.append(jnp.dot(kvtm[GR * g:GR * (g + 1), lo:lo + _PHI_W], phi[lo:lo + _PHI_W, :],
                                  preferred_element_type=jnp.float32))
        oT = jnp.concatenate(pieces, axis=0)
        o = oT.T.astype(jnp.bfloat16)
        x1 = x_scr[rows, :] + jnp.dot(o, wo_v[...], preferred_element_type=jnp.float32)
        xn1 = _layernorm_bf16(x1)
        h = jnp.dot(xn1, w1_v[...], preferred_element_type=jnp.float32)
        h = h * jax.nn.sigmoid(h)
        x2 = x1 + jnp.dot(h.astype(jnp.bfloat16), w2_v[...], preferred_element_type=jnp.float32)

        @pl.when(phase == 1)
        def _():
            x_scr[rows, :] = x2

        @pl.when(phase == 2)
        def _():
            o_ref[...] = x2.astype(o_ref.dtype)

    @pl.when(phase == 0)
    def _load_x():
        x_scr[rows, :] = x_ref[...].astype(jnp.float32)

    @pl.when(phase < 2)
    def _part_a():
        xn = _layernorm_bf16(x_scr[rows, :])
        pT = jax.lax.dot_general(wT[...], xn, _NT, preferred_element_type=jnp.float32)
        pq_scr[:, rows] = pT[0:D]
        vT = pT[2 * D:3 * D].astype(jnp.bfloat16)
        e1, e2, s1, s2 = _dual_softmax_parts(pT[D:2 * D])
        phik = _interleave_signs(e1 * (1.0 / s1), e2 * (1.0 / s2))
        zsum = phik[:, 0:128]
        for c in range(1, TB // 128):
            zsum = zsum + phik[:, 128 * c:128 * (c + 1)]
        zacc[...] += zsum
        phikb = phik.astype(jnp.bfloat16)
        for g in range(G):
            lo = _PHI_LO[g]
            kvt[GR * g:GR * (g + 1), lo:lo + _PHI_W] += jax.lax.dot_general(
                vT[GR * g:GR * (g + 1), :], phikb[lo:lo + _PHI_W, :], _NT,
                preferred_element_type=jnp.float32)


@jax.jit
def pallas_interleave_layers__linear_kernel_hedgehog__dense_activation_silu__prompt_kernel(
    A_x: jax.Array,
    A_wqkv: jax.Array,
    A_w_phi: jax.Array,
    A_wo: jax.Array,
    B_x: jax.Array,
    B_w1: jax.Array,
    B_w2: jax.Array,
):
    del B_x
    wphi2 = A_w_phi.reshape(D, DH)

    grid_spec = pltpu.PrefetchScalarGridSpec(
        num_scalar_prefetch=0,
        grid=(3, NB),
        in_specs=[
            pl.BlockSpec((None, TB, D), lambda p, i: (0, jnp.where(p == 0, i, NB - 1), 0)),
            pl.BlockSpec((D, DH), lambda p, i: (0, 0)),
            pl.BlockSpec(memory_space=pl.ANY),
            pl.BlockSpec(memory_space=pl.ANY),
            pl.BlockSpec(memory_space=pl.ANY),
            pl.BlockSpec(memory_space=pl.ANY),
        ],
        out_specs=pl.BlockSpec((None, TB, D), lambda p, i: (0, jnp.where(p == 2, i, 0), 0)),
        scratch_shapes=[
            pltpu.VMEM((D, 3 * D), jnp.bfloat16),
            pltpu.VMEM((D, D), jnp.bfloat16),
            pltpu.VMEM((D, F), jnp.bfloat16),
            pltpu.VMEM((F, D), jnp.bfloat16),
            pltpu.VMEM((3 * D, D), jnp.bfloat16),
            pltpu.VMEM((S, D), jnp.float32),
            pltpu.VMEM((D, S), jnp.float32),
            pltpu.VMEM((D, 2 * D), jnp.float32),
            pltpu.VMEM((D, 2 * D), jnp.bfloat16),
            pltpu.VMEM((2 * D, 128), jnp.float32),
            pltpu.VMEM((2 * D, TB), jnp.float32),
            pltpu.SemaphoreType.DMA((4,)),
        ],
    )
    return pl.pallas_call(
        _kernel,
        grid_spec=grid_spec,
        out_shape=jax.ShapeDtypeStruct(A_x.shape, A_x.dtype),
        compiler_params=pltpu.CompilerParams(
            dimension_semantics=("arbitrary", "arbitrary"),
            vmem_limit_bytes=100 * 1024 * 1024,
        ),
    )(A_x, wphi2, A_wqkv, A_wo, B_w1, B_w2)
```

```python
import jax
import jax.numpy as jnp
import jax.experimental.pallas as pl
import jax.experimental.pallas.tpu as pltpu

S = 2048
D = 640
H = 32
DH = D // H
F = 1728
G = 4
HG = H // G
GR = HG * DH
GA = GR + 16
TB = 512
NB = S // TB
LN_EPS = 1e-5
DEN_EPS = 1e-6

_NT = (((1,), (1,)), ((), ()))

_PHI_LO = tuple(128 * ((2 * GR * g) // 128) for g in range(G))
_PHI_W = 384
_QK_LO = tuple(128 * ((GR * g) // 128) for g in range(G))
_QK_W = 256


def _layernorm_bf16(x):
    m = jnp.mean(x, axis=-1, keepdims=True)
    xc = x - m
    v = jnp.mean(xc * xc, axis=-1, keepdims=True)
    return (xc * jax.lax.rsqrt(v + LN_EPS)).astype(jnp.bfloat16)


def _dual_softmax_parts(pT):
    p4 = pT.reshape(G, DH, HG, TB)
    mx = jnp.max(p4, axis=1, keepdims=True)
    mn = jnp.min(p4, axis=1, keepdims=True)
    e1 = jnp.exp(p4 - mx)
    e2 = jnp.exp(mn - p4)
    s1 = jnp.sum(e1, axis=1, keepdims=True)
    s2 = jnp.sum(e2, axis=1, keepdims=True)
    return e1, e2, s1, s2


def _interleave_signs(f1, f2):
    return jnp.stack([f1, f2], axis=1).reshape(2 * D, TB)


def _kernel(x_ref, wphi_ref, wqkv_hbm, wo_hbm, w1_hbm, w2_hbm, o_ref,
            wqkv_v, wo_v, w1_v, w2_v, wT, pm_scr, wo_p, x_scr, phiq_scr, kvt, kvtm, sems):
    phase = pl.program_id(0)
    i = pl.program_id(1)
    row0 = pl.multiple_of(i * TB, TB)
    rows = pl.ds(row0, TB)

    def weight_copy(k):
        src, dst = ((wqkv_hbm, wqkv_v), (wo_hbm, wo_v), (w1_hbm, w1_v), (w2_hbm, w2_v))[k]
        return pltpu.make_async_copy(src, dst, sems.at[k])

    @pl.when(jnp.logical_and(phase == 0, i == 0))
    def _prologue():
        for k in range(4):
            weight_copy(k).start()
        r_loc = jax.lax.broadcasted_iota(jnp.int32, (GR, 1), 0)
        hl_r = r_loc & (HG - 1)
        fd_r = r_loc >> 3
        f_iota = jax.lax.broadcasted_iota(jnp.int32, (GR, DH), 1)
        rep = (jax.lax.broadcasted_iota(jnp.int32, (GR, DH), 0) >> 3 == f_iota).astype(jnp.bfloat16)
        bds = []
        for g in range(G):
            lo = _QK_LO[g]
            j = lo + jax.lax.broadcasted_iota(jnp.int32, (1, _QK_W), 1)
            h_c = j // DH
            d_c = j - DH * h_c
            same_head = (h_c - HG * g) == hl_r
            bd_u = jax.lax.dot_general(rep, wphi_ref[lo:lo + _QK_W, :], _NT,
                                       preferred_element_type=jnp.float32)
            bds.append(jnp.where(same_head, bd_u, 0.0).astype(jnp.bfloat16))
            pm_scr[g] = jnp.where(jnp.logical_and(same_head, d_c == fd_r), 1.0, 0.0).astype(jnp.bfloat16)
        weight_copy(0).wait()
        for g in range(G):
            lo = _QK_LO[g]
            for part, lhs in enumerate((bds[g], bds[g], pm_scr[g])):
                w_g = wqkv_v[:, part * D + lo:part * D + lo + _QK_W]
                wT[part * D + GR * g:part * D + GR * (g + 1), :] = jax.lax.dot_general(
                    lhs, w_g, _NT, preferred_element_type=jnp.float32).astype(jnp.bfloat16)

    @pl.when(jnp.logical_and(phase == 1, i == 0))
    def _prepare_wo():
        for k in range(1, 4):
            weight_copy(k).wait()
        for g in range(G):
            lo = _QK_LO[g]
            wo_p[GR * g:GR * (g + 1), :] = jnp.dot(pm_scr[g], wo_v[lo:lo + _QK_W, :],
                                                   preferred_element_type=jnp.float32).astype(jnp.bfloat16)

    @pl.when(jnp.logical_and(phase > 0, i == 0))
    def _finalize_kv():
        hl_r = jax.lax.broadcasted_iota(jnp.int32, (GA, 1), 0) & (HG - 1)
        cw = jax.lax.broadcasted_iota(jnp.int32, (1, _PHI_W), 1)
        for g in range(G):
            col = _PHI_LO[g] + cw
            in_group = jnp.logical_and(col >= 2 * GR * g, col < 2 * GR * (g + 1))
            keep = jnp.logical_and(in_group, (cw & (HG - 1)) == hl_r)
            kvtm[g] = jnp.where(keep, kvt[g], 0.0).astype(jnp.bfloat16)

    @pl.when(jnp.logical_and(phase < 2, i == 0))
    def _zero_acc():
        kvt[...] = jnp.zeros_like(kvt)

    def part_a(x):
        xn = _layernorm_bf16(x)
        pT = jax.lax.dot_general(wT[...], xn, _NT, preferred_element_type=jnp.float32)
        e1, e2, s1, s2 = _dual_softmax_parts(pT[0:D])
        phiq_scr[:, rows] = _interleave_signs(e1 * (1.0 / s1), e2 * (1.0 / s2)).astype(jnp.bfloat16)
        e1, e2, s1, s2 = _dual_softmax_parts(pT[D:2 * D])
        phik = _interleave_signs(e1 * (1.0 / s1), e2 * (1.0 / s2)).astype(jnp.bfloat16)
        ones = jnp.ones((GA - GR, TB), jnp.bfloat16)
        for g in range(G):
            lo = _PHI_LO[g]
            v_aug = jnp.concatenate(
                [pT[2 * D + GR * g:2 * D + GR * (g + 1)].astype(jnp.bfloat16), ones], axis=0)
            kvt[g] += jax.lax.dot_general(v_aug, phik[lo:lo + _PHI_W, :], _NT,
                                          preferred_element_type=jnp.float32)

    def part_b():
        phiq = phiq_scr[:, rows]
        pieces = []
        for g in range(G):
            lo = _PHI_LO[g]
            res = jnp.dot(kvtm[g], phiq[lo:lo + _PHI_W, :], preferred_element_type=jnp.float32)
            den = res[GR:GR + HG] + DEN_EPS
            o_g = res[0:GR].reshape(DH, HG, TB) * (1.0 / den)[None]
            pieces.append(o_g.reshape(GR, TB))
        oT = jnp.concatenate(pieces, axis=0)
        o = oT.T.astype(jnp.bfloat16)
        x1 = x_scr[rows, :] + jnp.dot(o, wo_p[...], preferred_element_type=jnp.float32)
        xn1 = _layernorm_bf16(x1)
        h = jax.lax.dot_general(xn1, w1_v[...], _NT, preferred_element_type=jnp.float32)
        h = h * jax.nn.sigmoid(h)
        return x1 + jnp.dot(h.astype(jnp.bfloat16), w2_v[...], preferred_element_type=jnp.float32)

    @pl.when(phase == 0)
    def _load_x():
        x_scr[rows, :] = x_ref[...].astype(jnp.float32)

    @pl.when(phase > 0)
    def _run_b():
        x2 = part_b()

        @pl.when(phase == 1)
        def _():
            x_scr[rows, :] = x2

        @pl.when(phase == 2)
        def _():
            o_ref[...] = x2.astype(o_ref.dtype)

    @pl.when(phase < 2)
    def _run_a():
        part_a(x_scr[rows, :])


@jax.jit
def pallas_interleave_layers__linear_kernel_hedgehog__dense_activation_silu__prompt_kernel(
    A_x: jax.Array,
    A_wqkv: jax.Array,
    A_w_phi: jax.Array,
    A_wo: jax.Array,
    B_x: jax.Array,
    B_w1: jax.Array,
    B_w2: jax.Array,
):
    del B_x
    wphi2 = A_w_phi.reshape(D, DH)
    w1_t = B_w1.T

    grid_spec = pltpu.PrefetchScalarGridSpec(
        num_scalar_prefetch=0,
        grid=(3, NB),
        in_specs=[
            pl.BlockSpec((None, TB, D), lambda p, i: (0, jnp.where(p == 0, i, NB - 1), 0)),
            pl.BlockSpec((D, DH), lambda p, i: (0, 0)),
            pl.BlockSpec(memory_space=pl.ANY),
            pl.BlockSpec(memory_space=pl.ANY),
            pl.BlockSpec(memory_space=pl.ANY),
            pl.BlockSpec(memory_space=pl.ANY),
        ],
        out_specs=pl.BlockSpec((None, TB, D), lambda p, i: (0, jnp.where(p == 2, i, 0), 0)),
        scratch_shapes=[
            pltpu.VMEM((D, 3 * D), jnp.bfloat16),
            pltpu.VMEM((D, D), jnp.bfloat16),
            pltpu.VMEM((F, D), jnp.bfloat16),
            pltpu.VMEM((F, D), jnp.bfloat16),
            pltpu.VMEM((3 * D, D), jnp.bfloat16),
            pltpu.VMEM((G, GR, _QK_W), jnp.bfloat16),
            pltpu.VMEM((D, D), jnp.bfloat16),
            pltpu.VMEM((S, D), jnp.float32),
            pltpu.VMEM((2 * D, S), jnp.bfloat16),
            pltpu.VMEM((G, GA, _PHI_W), jnp.float32),
            pltpu.VMEM((G, GA, _PHI_W), jnp.bfloat16),
            pltpu.SemaphoreType.DMA((4,)),
        ],
    )
    return pl.pallas_call(
        _kernel,
        grid_spec=grid_spec,
        out_shape=jax.ShapeDtypeStruct(A_x.shape, A_x.dtype),
        compiler_params=pltpu.CompilerParams(
            dimension_semantics=("arbitrary", "arbitrary"),
            vmem_limit_bytes=100 * 1024 * 1024,
        ),
    )(A_x, wphi2, A_wqkv, A_wo, w1_t, B_w2)
```

```python
import jax
import jax.numpy as jnp
import jax.experimental.pallas as pl
import jax.experimental.pallas.tpu as pltpu

S = 2048
D = 640
H = 32
DH = D // H
F = 1728
G = 4
HG = H // G
GR = HG * DH
GA = GR + 16
TB = 512
NB = S // TB
LN_EPS = 1e-5
DEN_EPS = 1e-6

_NT = (((1,), (1,)), ((), ()))

_PHI_LO = tuple(128 * ((2 * GR * g) // 128) for g in range(G))
_PHI_W = 384
_QK_LO = tuple(128 * ((GR * g) // 128) for g in range(G))
_QK_W = 256


def _layernorm_bf16(x):
    m = jnp.mean(x, axis=-1, keepdims=True)
    xc = x - m
    v = jnp.mean(xc * xc, axis=-1, keepdims=True)
    return (xc * jax.lax.rsqrt(v + LN_EPS)).astype(jnp.bfloat16)


def _dual_softmax_parts(pT):
    p4 = pT.reshape(G, DH, HG, TB)
    mx = jnp.max(p4, axis=1, keepdims=True)
    mn = jnp.min(p4, axis=1, keepdims=True)
    e1 = jnp.exp(p4 - mx)
    e2 = jnp.exp(mn - p4)
    s1 = jnp.sum(e1, axis=1, keepdims=True)
    s2 = jnp.sum(e2, axis=1, keepdims=True)
    return e1, e2, s1, s2


def _interleave_signs(f1, f2):
    return jnp.stack([f1, f2], axis=1).reshape(2 * D, TB)


def _kernel(x_ref, wphi_ref, wqkv_hbm, wo_hbm, w1_hbm, w2_hbm, o_ref,
            wqkv_v, wo_v, w1_v, w2_v, wT, pm_scr, wo_p, x_scr, phiq_scr, kvt, kvtm, sems):
    phase = pl.program_id(0)
    i = pl.program_id(1)
    row0 = pl.multiple_of(i * TB, TB)
    rows = pl.ds(row0, TB)

    def qkv_copy(part):
        cols = pl.ds(part * D, D)
        return pltpu.make_async_copy(wqkv_hbm.at[:, cols], wqkv_v.at[:, cols], sems.at[part])

    def weight_copy(k):
        src, dst = ((wo_hbm, wo_v), (w1_hbm, w1_v), (w2_hbm, w2_v))[k]
        return pltpu.make_async_copy(src, dst, sems.at[3 + k])

    @pl.when(jnp.logical_and(phase == 0, i == 0))
    def _prologue():
        for part in range(3):
            qkv_copy(part).start()
        r_loc = jax.lax.broadcasted_iota(jnp.int32, (GR, 1), 0)
        hl_r = r_loc & (HG - 1)
        fd_r = r_loc >> 3
        f_iota = jax.lax.broadcasted_iota(jnp.int32, (GR, DH), 1)
        rep = (jax.lax.broadcasted_iota(jnp.int32, (GR, DH), 0) >> 3 == f_iota).astype(jnp.bfloat16)
        bds = []
        for g in range(G):
            lo = _QK_LO[g]
            j = lo + jax.lax.broadcasted_iota(jnp.int32, (1, _QK_W), 1)
            h_c = j // DH
            d_c = j - DH * h_c
            same_head = (h_c - HG * g) == hl_r
            bd_u = jax.lax.dot_general(rep, wphi_ref[lo:lo + _QK_W, :], _NT,
                                       preferred_element_type=jnp.float32)
            bds.append(jnp.where(same_head, bd_u, 0.0).astype(jnp.bfloat16))
            pm_scr[g] = jnp.where(jnp.logical_and(same_head, d_c == fd_r), 1.0, 0.0).astype(jnp.bfloat16)
        for part in range(3):
            qkv_copy(part).wait()
            if part == 0:
                for k in range(3):
                    weight_copy(k).start()
            for g in range(G):
                lo = _QK_LO[g]
                lhs = pm_scr[g] if part == 2 else bds[g]
                w_g = wqkv_v[:, part * D + lo:part * D + lo + _QK_W]
                wT[part * D + GR * g:part * D + GR * (g + 1), :] = jax.lax.dot_general(
                    lhs, w_g, _NT, preferred_element_type=jnp.float32).astype(jnp.bfloat16)

    @pl.when(jnp.logical_and(phase == 1, i == 0))
    def _prepare_wo():
        for k in range(3):
            weight_copy(k).wait()
        for g in range(G):
            lo = _QK_LO[g]
            wo_p[GR * g:GR * (g + 1), :] = jnp.dot(pm_scr[g], wo_v[lo:lo + _QK_W, :],
                                                   preferred_element_type=jnp.float32).astype(jnp.bfloat16)

    @pl.when(jnp.logical_and(phase > 0, i == 0))
    def _finalize_kv():
        hl_r = jax.lax.broadcasted_iota(jnp.int32, (GA, 1), 0) & (HG - 1)
        cw = jax.lax.broadcasted_iota(jnp.int32, (1, _PHI_W), 1)
        for g in range(G):
            col = _PHI_LO[g] + cw
            in_group = jnp.logical_and(col >= 2 * GR * g, col < 2 * GR * (g + 1))
            keep = jnp.logical_and(in_group, (cw & (HG - 1)) == hl_r)
            kvtm[g] = jnp.where(keep, kvt[g], 0.0).astype(jnp.bfloat16)

    @pl.when(jnp.logical_and(phase < 2, i == 0))
    def _zero_acc():
        kvt[...] = jnp.zeros_like(kvt)

    def part_a(x):
        xn = _layernorm_bf16(x)
        pT = jax.lax.dot_general(wT[...], xn, _NT, preferred_element_type=jnp.float32)
        e1, e2, s1, s2 = _dual_softmax_parts(pT[0:D])
        phiq_scr[:, rows] = _interleave_signs(e1 * (1.0 / s1), e2 * (1.0 / s2)).astype(jnp.bfloat16)
        e1, e2, s1, s2 = _dual_softmax_parts(pT[D:2 * D])
        phik = _interleave_signs(e1 * (1.0 / s1), e2 * (1.0 / s2)).astype(jnp.bfloat16)
        ones = jnp.ones((GA - GR, TB), jnp.bfloat16)
        for g in range(G):
            lo = _PHI_LO[g]
            v_aug = jnp.concatenate(
                [pT[2 * D + GR * g:2 * D + GR * (g + 1)].astype(jnp.bfloat16), ones], axis=0)
            kvt[g] += jax.lax.dot_general(v_aug, phik[lo:lo + _PHI_W, :], _NT,
                                          preferred_element_type=jnp.float32)

    def part_b():
        phiq = phiq_scr[:, rows]
        pieces = []
        for g in range(G):
            lo = _PHI_LO[g]
            res = jnp.dot(kvtm[g], phiq[lo:lo + _PHI_W, :], preferred_element_type=jnp.float32)
            den = res[GR:GR + HG] + DEN_EPS
            o_g = res[0:GR].reshape(DH, HG, TB) * (1.0 / den)[None]
            pieces.append(o_g.reshape(GR, TB))
        oT = jnp.concatenate(pieces, axis=0)
        o = oT.T.astype(jnp.bfloat16)
        x1 = x_scr[rows, :] + jnp.dot(o, wo_p[...], preferred_element_type=jnp.float32)
        xn1 = _layernorm_bf16(x1)
        h = jax.lax.dot_general(xn1, w1_v[...], _NT, preferred_element_type=jnp.float32)
        h = h * jax.nn.sigmoid(h)
        return x1 + jnp.dot(h.astype(jnp.bfloat16), w2_v[...], preferred_element_type=jnp.float32)

    @pl.when(phase == 0)
    def _load_x():
        x_scr[rows, :] = x_ref[...].astype(jnp.float32)

    @pl.when(phase > 0)
    def _run_b():
        x2 = part_b()

        @pl.when(phase == 1)
        def _():
            x_scr[rows, :] = x2

        @pl.when(phase == 2)
        def _():
            o_ref[...] = x2.astype(o_ref.dtype)

    @pl.when(phase < 2)
    def _run_a():
        part_a(x_scr[rows, :])


@jax.jit
def pallas_interleave_layers__linear_kernel_hedgehog__dense_activation_silu__prompt_kernel(
    A_x: jax.Array,
    A_wqkv: jax.Array,
    A_w_phi: jax.Array,
    A_wo: jax.Array,
    B_x: jax.Array,
    B_w1: jax.Array,
    B_w2: jax.Array,
):
    del B_x
    wphi2 = A_w_phi.reshape(D, DH)
    w1_t = B_w1.T

    grid_spec = pltpu.PrefetchScalarGridSpec(
        num_scalar_prefetch=0,
        grid=(3, NB),
        in_specs=[
            pl.BlockSpec((None, TB, D), lambda p, i: (0, jnp.where(p == 0, i, NB - 1), 0)),
            pl.BlockSpec((D, DH), lambda p, i: (0, 0)),
            pl.BlockSpec(memory_space=pl.ANY),
            pl.BlockSpec(memory_space=pl.ANY),
            pl.BlockSpec(memory_space=pl.ANY),
            pl.BlockSpec(memory_space=pl.ANY),
        ],
        out_specs=pl.BlockSpec((None, TB, D), lambda p, i: (0, jnp.where(p == 2, i, 0), 0)),
        scratch_shapes=[
            pltpu.VMEM((D, 3 * D), jnp.bfloat16),
            pltpu.VMEM((D, D), jnp.bfloat16),
            pltpu.VMEM((F, D), jnp.bfloat16),
            pltpu.VMEM((F, D), jnp.bfloat16),
            pltpu.VMEM((3 * D, D), jnp.bfloat16),
            pltpu.VMEM((G, GR, _QK_W), jnp.bfloat16),
            pltpu.VMEM((D, D), jnp.bfloat16),
            pltpu.VMEM((S, D), jnp.float32),
            pltpu.VMEM((2 * D, S), jnp.bfloat16),
            pltpu.VMEM((G, GA, _PHI_W), jnp.float32),
            pltpu.VMEM((G, GA, _PHI_W), jnp.bfloat16),
            pltpu.SemaphoreType.DMA((6,)),
        ],
    )
    return pl.pallas_call(
        _kernel,
        grid_spec=grid_spec,
        out_shape=jax.ShapeDtypeStruct(A_x.shape, A_x.dtype),
        compiler_params=pltpu.CompilerParams(
            dimension_semantics=("arbitrary", "arbitrary"),
            vmem_limit_bytes=100 * 1024 * 1024,
        ),
    )(A_x, wphi2, A_wqkv, A_wo, w1_t, B_w2)
```

```python
import jax
import jax.numpy as jnp
import jax.experimental.pallas as pl
import jax.experimental.pallas.tpu as pltpu

S = 2048
D = 640
H = 32
DH = D // H
F = 1728
G = 4
HG = H // G
GR = HG * DH
GA = GR + 16
TB = 512
NB = S // TB
LN_EPS = 1e-5
DEN_EPS = 1e-6

_NT = (((1,), (1,)), ((), ()))

_PHI_LO = tuple(128 * ((2 * GR * g) // 128) for g in range(G))
_PHI_W = 384
_QK_LO = tuple(128 * ((GR * g) // 128) for g in range(G))
_QK_W = 256


def _layernorm_bf16(x):
    m = jnp.mean(x, axis=-1, keepdims=True)
    xc = x - m
    v = jnp.mean(xc * xc, axis=-1, keepdims=True)
    return (xc * jax.lax.rsqrt(v + LN_EPS)).astype(jnp.bfloat16)


def _dual_softmax_parts(pT):
    p4 = pT.reshape(G, DH, HG, TB)
    mx = jnp.max(p4, axis=1, keepdims=True)
    mn = jnp.min(p4, axis=1, keepdims=True)
    e1 = jnp.exp(p4 - mx)
    e2 = jnp.exp(mn - p4)
    s1 = jnp.sum(e1, axis=1, keepdims=True)
    s2 = jnp.sum(e2, axis=1, keepdims=True)
    return e1, e2, s1, s2


def _interleave_signs(f1, f2):
    return jnp.stack([f1, f2], axis=1).reshape(2 * D, TB)


def _kernel(x_hbm, wphi_ref, wqkv_hbm, wo_hbm, w1_hbm, w2_hbm, o_hbm,
            wqkv_v, wo_v, w1_v, w2_v, wT, pm_scr, wo_p, x_scr, w1sum, phiq_scr, kvt, kvtm, sems):
    phase = pl.program_id(0)
    i = pl.program_id(1)
    row0 = pl.multiple_of(i * TB, TB)
    rows = pl.ds(row0, TB)

    def qkv_copy(part):
        cols = pl.ds(part * D, D)
        return pltpu.make_async_copy(wqkv_hbm.at[:, cols], wqkv_v.at[:, cols], sems.at[part])

    def weight_copy(k):
        src, dst = ((wo_hbm, wo_v), (w1_hbm, w1_v), (w2_hbm, w2_v))[k]
        return pltpu.make_async_copy(src, dst, sems.at[3 + k])

    def x_in_copy(j):
        blk = pl.ds(j * TB, TB)
        return pltpu.make_async_copy(x_hbm.at[blk, :], x_scr.at[blk, :], sems.at[6 + j])

    def x_out_copy(j):
        blk = pl.ds(j * TB, TB)
        return pltpu.make_async_copy(x_scr.at[blk, :], o_hbm.at[blk, :], sems.at[6 + NB + j])

    @pl.when(jnp.logical_and(phase == 0, i == 0))
    def _prologue():
        for part in range(3):
            qkv_copy(part).start()
        for j in range(NB):
            x_in_copy(j).start()
        r_loc = jax.lax.broadcasted_iota(jnp.int32, (GR, 1), 0)
        hl_r = r_loc & (HG - 1)
        fd_r = r_loc >> 3
        f_iota = jax.lax.broadcasted_iota(jnp.int32, (GR, DH), 1)
        rep = (jax.lax.broadcasted_iota(jnp.int32, (GR, DH), 0) >> 3 == f_iota).astype(jnp.bfloat16)
        bds = []
        for g in range(G):
            lo = _QK_LO[g]
            j = lo + jax.lax.broadcasted_iota(jnp.int32, (1, _QK_W), 1)
            h_c = j // DH
            d_c = j - DH * h_c
            same_head = (h_c - HG * g) == hl_r
            bd_u = jax.lax.dot_general(rep, wphi_ref[lo:lo + _QK_W, :], _NT,
                                       preferred_element_type=jnp.float32)
            bds.append(jnp.where(same_head, bd_u, 0.0).astype(jnp.bfloat16))
            pm_scr[g] = jnp.where(jnp.logical_and(same_head, d_c == fd_r), 1.0, 0.0).astype(jnp.bfloat16)
        for part in range(3):
            qkv_copy(part).wait()
            if part == 0:
                for k in range(3):
                    weight_copy(k).start()
            for g in range(G):
                lo = _QK_LO[g]
                lhs = pm_scr[g] if part == 2 else bds[g]
                w_g = wqkv_v[:, part * D + lo:part * D + lo + _QK_W]
                wT[part * D + GR * g:part * D + GR * (g + 1), :] = jax.lax.dot_general(
                    lhs, w_g, _NT, preferred_element_type=jnp.float32).astype(jnp.bfloat16)

    @pl.when(jnp.logical_and(phase == 1, i == 0))
    def _prepare_wo():
        for k in range(3):
            weight_copy(k).wait()
        for g in range(G):
            lo = _QK_LO[g]
            wo_p[GR * g:GR * (g + 1), :] = jnp.dot(pm_scr[g], wo_v[lo:lo + _QK_W, :],
                                                   preferred_element_type=jnp.float32).astype(jnp.bfloat16)
        w1sum[...] = jax.lax.dot_general(jnp.ones((HG, D), jnp.bfloat16), w1_v[...], _NT,
                                         preferred_element_type=jnp.float32)

    @pl.when(jnp.logical_and(phase > 0, i == 0))
    def _finalize_kv():
        hl_r = jax.lax.broadcasted_iota(jnp.int32, (GA, 1), 0) & (HG - 1)
        cw = jax.lax.broadcasted_iota(jnp.int32, (1, _PHI_W), 1)
        for g in range(G):
            col = _PHI_LO[g] + cw
            in_group = jnp.logical_and(col >= 2 * GR * g, col < 2 * GR * (g + 1))
            keep = jnp.logical_and(in_group, (cw & (HG - 1)) == hl_r)
            kvtm[g] = jnp.where(keep, kvt[g], 0.0).astype(jnp.bfloat16)

    @pl.when(jnp.logical_and(phase < 2, i == 0))
    def _zero_acc():
        kvt[...] = jnp.zeros_like(kvt)

    def part_a(x):
        xn = _layernorm_bf16(x)
        pT = jax.lax.dot_general(wT[...], xn, _NT, preferred_element_type=jnp.float32)
        e1, e2, s1, s2 = _dual_softmax_parts(pT[0:D])
        phiq_scr[:, rows] = _interleave_signs(e1 * (1.0 / s1), e2 * (1.0 / s2)).astype(jnp.bfloat16)
        e1, e2, s1, s2 = _dual_softmax_parts(pT[D:2 * D])
        phik = _interleave_signs(e1 * (1.0 / s1), e2 * (1.0 / s2)).astype(jnp.bfloat16)
        ones = jnp.ones((GA - GR, TB), jnp.bfloat16)
        for g in range(G):
            lo = _PHI_LO[g]
            v_aug = jnp.concatenate(
                [pT[2 * D + GR * g:2 * D + GR * (g + 1)].astype(jnp.bfloat16), ones], axis=0)
            kvt[g] += jax.lax.dot_general(v_aug, phik[lo:lo + _PHI_W, :], _NT,
                                          preferred_element_type=jnp.float32)

    def part_b():
        phiq = phiq_scr[:, rows]
        pieces = []
        for g in range(G):
            lo = _PHI_LO[g]
            res = jnp.dot(kvtm[g], phiq[lo:lo + _PHI_W, :], preferred_element_type=jnp.float32)
            den = res[GR:GR + HG] + DEN_EPS
            o_g = res[0:GR].reshape(DH, HG, TB) * (1.0 / den)[None]
            pieces.append(o_g.reshape(GR, TB))
        oT = jnp.concatenate(pieces, axis=0)
        o = oT.T.astype(jnp.bfloat16)
        x1 = x_scr[rows, :].astype(jnp.float32) + jnp.dot(o, wo_p[...], preferred_element_type=jnp.float32)
        h = jax.lax.dot_general(x1.astype(jnp.bfloat16), w1_v[...], _NT,
                                preferred_element_type=jnp.float32)
        m = jnp.mean(x1, axis=-1, keepdims=True)
        xc = x1 - m
        rstd = jax.lax.rsqrt(jnp.mean(xc * xc, axis=-1, keepdims=True) + LN_EPS)
        h = (h - m * w1sum[0:1, :]) * rstd
        h = h * jax.nn.sigmoid(h)
        return x1 + jnp.dot(h.astype(jnp.bfloat16), w2_v[...], preferred_element_type=jnp.float32)

    @pl.when(phase == 0)
    def _wait_x():
        x_in_copy(i).wait()

    @pl.when(phase > 0)
    def _run_b():
        x_scr[rows, :] = part_b().astype(jnp.bfloat16)

    @pl.when(phase == 2)
    def _write_out():
        x_out_copy(i).start()

    @pl.when(jnp.logical_and(phase == 2, i == NB - 1))
    def _drain_out():
        for j in range(NB):
            x_out_copy(j).wait()

    @pl.when(phase < 2)
    def _run_a():
        part_a(x_scr[rows, :].astype(jnp.float32))


@jax.jit
def pallas_interleave_layers__linear_kernel_hedgehog__dense_activation_silu__prompt_kernel(
    A_x: jax.Array,
    A_wqkv: jax.Array,
    A_w_phi: jax.Array,
    A_wo: jax.Array,
    B_x: jax.Array,
    B_w1: jax.Array,
    B_w2: jax.Array,
):
    del B_x
    wphi2 = A_w_phi.reshape(D, DH)
    w1_t = B_w1.T

    grid_spec = pltpu.PrefetchScalarGridSpec(
        num_scalar_prefetch=0,
        grid=(3, NB),
        in_specs=[
            pl.BlockSpec(memory_space=pl.ANY),
            pl.BlockSpec((D, DH), lambda p, i: (0, 0)),
            pl.BlockSpec(memory_space=pl.ANY),
            pl.BlockSpec(memory_space=pl.ANY),
            pl.BlockSpec(memory_space=pl.ANY),
            pl.BlockSpec(memory_space=pl.ANY),
        ],
        out_specs=pl.BlockSpec(memory_space=pl.ANY),
        scratch_shapes=[
            pltpu.VMEM((D, 3 * D), jnp.bfloat16),
            pltpu.VMEM((D, D), jnp.bfloat16),
            pltpu.VMEM((F, D), jnp.bfloat16),
            pltpu.VMEM((F, D), jnp.bfloat16),
            pltpu.VMEM((3 * D, D), jnp.bfloat16),
            pltpu.VMEM((G, GR, _QK_W), jnp.bfloat16),
            pltpu.VMEM((D, D), jnp.bfloat16),
            pltpu.VMEM((S, D), jnp.bfloat16),
            pltpu.VMEM((HG, F), jnp.float32),
            pltpu.VMEM((2 * D, S), jnp.bfloat16),
            pltpu.VMEM((G, GA, _PHI_W), jnp.float32),
            pltpu.VMEM((G, GA, _PHI_W), jnp.bfloat16),
            pltpu.SemaphoreType.DMA((6 + 2 * NB,)),
        ],
    )
    return pl.pallas_call(
        _kernel,
        grid_spec=grid_spec,
        out_shape=jax.ShapeDtypeStruct((S, D), A_x.dtype),
        compiler_params=pltpu.CompilerParams(
            dimension_semantics=("arbitrary", "arbitrary"),
            vmem_limit_bytes=100 * 1024 * 1024,
        ),
    )(A_x.reshape(S, D), wphi2, A_wqkv, A_wo, w1_t, B_w2).reshape(A_x.shape)
```

```python
import jax
import jax.numpy as jnp
import jax.experimental.pallas as pl
import jax.experimental.pallas.tpu as pltpu

S = 2048
D = 640
H = 32
DH = D // H
F = 1728
G = 4
HG = H // G
GR = HG * DH
GA = GR + 16
TB = 512
NB = S // TB
LN_EPS = 1e-5
DEN_EPS = 1e-6

_NT = (((1,), (1,)), ((), ()))

_PHI_LO = tuple(128 * ((2 * GR * g) // 128) for g in range(G))
_PHI_W = 384
_QK_LO = tuple(128 * ((GR * g) // 128) for g in range(G))
_QK_W = 256


def _layernorm_bf16(x):
    m = jnp.mean(x, axis=-1, keepdims=True)
    xc = x - m
    v = jnp.mean(xc * xc, axis=-1, keepdims=True)
    return (xc * jax.lax.rsqrt(v + LN_EPS)).astype(jnp.bfloat16)


def _dual_softmax_parts(pT):
    p4 = pT.reshape(G, DH, HG, TB)
    mx = jnp.max(p4, axis=1, keepdims=True)
    mn = jnp.min(p4, axis=1, keepdims=True)
    e1 = jnp.exp(p4 - mx)
    e2 = jnp.exp(mn - p4)
    s1 = jnp.sum(e1, axis=1, keepdims=True)
    s2 = jnp.sum(e2, axis=1, keepdims=True)
    return e1, e2, s1, s2


def _interleave_signs(f1, f2):
    return jnp.stack([f1, f2], axis=1).reshape(2 * D, TB)


def _kernel(x_hbm, wphi_ref, wqkv_hbm, wo_hbm, w1_hbm, w2_hbm, o_hbm,
            wqkv_v, wo_v, w1_v, w2_v, wT, pm_scr, wo_p, x_scr, phiq_scr, kvt, kvtm, sems):
    phase = pl.program_id(0)
    i = pl.program_id(1)
    row0 = pl.multiple_of(i * TB, TB)
    rows = pl.ds(row0, TB)

    def qkv_copy(part):
        cols = pl.ds(part * D, D)
        return pltpu.make_async_copy(wqkv_hbm.at[:, cols], wqkv_v.at[:, cols], sems.at[part])

    def weight_copy(k):
        src, dst = ((wo_hbm, wo_v), (w1_hbm, w1_v), (w2_hbm, w2_v))[k]
        return pltpu.make_async_copy(src, dst, sems.at[3 + k])

    def x_in_copy(j):
        blk = pl.ds(j * TB, TB)
        return pltpu.make_async_copy(x_hbm.at[blk, :], x_scr.at[blk, :], sems.at[6 + j])

    def x_out_copy(j):
        blk = pl.ds(j * TB, TB)
        return pltpu.make_async_copy(x_scr.at[blk, :], o_hbm.at[blk, :], sems.at[6 + NB + j])

    @pl.when(jnp.logical_and(phase == 0, i == 0))
    def _prologue():
        for part in range(3):
            qkv_copy(part).start()
        for j in range(NB):
            x_in_copy(j).start()
        r_loc = jax.lax.broadcasted_iota(jnp.int32, (GR, 1), 0)
        hl_r = r_loc & (HG - 1)
        fd_r = r_loc >> 3
        f_iota = jax.lax.broadcasted_iota(jnp.int32, (GR, DH), 1)
        rep = (jax.lax.broadcasted_iota(jnp.int32, (GR, DH), 0) >> 3 == f_iota).astype(jnp.bfloat16)
        bds = []
        for g in range(G):
            lo = _QK_LO[g]
            j = lo + jax.lax.broadcasted_iota(jnp.int32, (1, _QK_W), 1)
            h_c = j // DH
            d_c = j - DH * h_c
            same_head = (h_c - HG * g) == hl_r
            bd_u = jax.lax.dot_general(rep, wphi_ref[lo:lo + _QK_W, :], _NT,
                                       preferred_element_type=jnp.float32)
            bds.append(jnp.where(same_head, bd_u, 0.0).astype(jnp.bfloat16))
            pm_scr[g] = jnp.where(jnp.logical_and(same_head, d_c == fd_r), 1.0, 0.0).astype(jnp.bfloat16)
        for part in range(3):
            qkv_copy(part).wait()
            if part == 0:
                for k in range(3):
                    weight_copy(k).start()
            for g in range(G):
                lo = _QK_LO[g]
                lhs = pm_scr[g] if part == 2 else bds[g]
                w_g = wqkv_v[:, part * D + lo:part * D + lo + _QK_W]
                wT[part * D + GR * g:part * D + GR * (g + 1), :] = jax.lax.dot_general(
                    lhs, w_g, _NT, preferred_element_type=jnp.float32).astype(jnp.bfloat16)

    @pl.when(jnp.logical_and(phase == 1, i == 0))
    def _prepare_wo():
        for k in range(3):
            weight_copy(k).wait()
        for g in range(G):
            lo = _QK_LO[g]
            wo_p[GR * g:GR * (g + 1), :] = jnp.dot(pm_scr[g], wo_v[lo:lo + _QK_W, :],
                                                   preferred_element_type=jnp.float32).astype(jnp.bfloat16)

    @pl.when(jnp.logical_and(phase > 0, i == 0))
    def _finalize_kv():
        hl_r = jax.lax.broadcasted_iota(jnp.int32, (GA, 1), 0) & (HG - 1)
        cw = jax.lax.broadcasted_iota(jnp.int32, (1, _PHI_W), 1)
        for g in range(G):
            col = _PHI_LO[g] + cw
            in_group = jnp.logical_and(col >= 2 * GR * g, col < 2 * GR * (g + 1))
            keep = jnp.logical_and(in_group, (cw & (HG - 1)) == hl_r)
            kvtm[g] = jnp.where(keep, kvt[g], 0.0).astype(jnp.bfloat16)

    @pl.when(jnp.logical_and(phase < 2, i == 0))
    def _zero_acc():
        kvt[...] = jnp.zeros_like(kvt)

    def part_a(x):
        xn = _layernorm_bf16(x)
        pT = jax.lax.dot_general(wT[...], xn, _NT, preferred_element_type=jnp.float32)
        e1, e2, s1, s2 = _dual_softmax_parts(pT[0:D])
        phiq_scr[:, rows] = _interleave_signs(e1 * (1.0 / s1), e2 * (1.0 / s2)).astype(jnp.bfloat16)
        e1, e2, s1, s2 = _dual_softmax_parts(pT[D:2 * D])
        phik = _interleave_signs(e1 * (1.0 / s1), e2 * (1.0 / s2)).astype(jnp.bfloat16)
        ones = jnp.ones((GA - GR, TB), jnp.bfloat16)
        for g in range(G):
            lo = _PHI_LO[g]
            v_aug = jnp.concatenate(
                [pT[2 * D + GR * g:2 * D + GR * (g + 1)].astype(jnp.bfloat16), ones], axis=0)
            kvt[g] += jax.lax.dot_general(v_aug, phik[lo:lo + _PHI_W, :], _NT,
                                          preferred_element_type=jnp.float32)

    def part_b():
        phiq = phiq_scr[:, rows]
        pieces = []
        for g in range(G):
            lo = _PHI_LO[g]
            res = jnp.dot(kvtm[g], phiq[lo:lo + _PHI_W, :], preferred_element_type=jnp.float32)
            den = res[GR:GR + HG] + DEN_EPS
            o_g = res[0:GR].reshape(DH, HG, TB) * (1.0 / den)[None]
            pieces.append(o_g.reshape(GR, TB))
        oT = jnp.concatenate(pieces, axis=0)
        o = oT.T.astype(jnp.bfloat16)
        x1 = x_scr[rows, :].astype(jnp.float32) + jnp.dot(o, wo_p[...], preferred_element_type=jnp.float32)
        m = jnp.mean(x1, axis=-1, keepdims=True)
        xc = x1 - m
        h = jax.lax.dot_general(xc.astype(jnp.bfloat16), w1_v[...], _NT,
                                preferred_element_type=jnp.float32)
        h = h * jax.lax.rsqrt(jnp.mean(xc * xc, axis=-1, keepdims=True) + LN_EPS)
        h = h * jax.nn.sigmoid(h)
        return x1 + jnp.dot(h.astype(jnp.bfloat16), w2_v[...], preferred_element_type=jnp.float32)

    @pl.when(phase == 0)
    def _wait_x():
        x_in_copy(i).wait()

    @pl.when(phase > 0)
    def _run_b():
        x_scr[rows, :] = part_b().astype(jnp.bfloat16)

    @pl.when(phase == 2)
    def _write_out():
        x_out_copy(i).start()

    @pl.when(jnp.logical_and(phase == 2, i == NB - 1))
    def _drain_out():
        for j in range(NB):
            x_out_copy(j).wait()

    @pl.when(phase < 2)
    def _run_a():
        part_a(x_scr[rows, :].astype(jnp.float32))


@jax.jit
def pallas_interleave_layers__linear_kernel_hedgehog__dense_activation_silu__prompt_kernel(
    A_x: jax.Array,
    A_wqkv: jax.Array,
    A_w_phi: jax.Array,
    A_wo: jax.Array,
    B_x: jax.Array,
    B_w1: jax.Array,
    B_w2: jax.Array,
):
    del B_x
    wphi2 = A_w_phi.reshape(D, DH)
    w1_t = B_w1.T

    grid_spec = pltpu.PrefetchScalarGridSpec(
        num_scalar_prefetch=0,
        grid=(3, NB),
        in_specs=[
            pl.BlockSpec(memory_space=pl.ANY),
            pl.BlockSpec((D, DH), lambda p, i: (0, 0)),
            pl.BlockSpec(memory_space=pl.ANY),
            pl.BlockSpec(memory_space=pl.ANY),
            pl.BlockSpec(memory_space=pl.ANY),
            pl.BlockSpec(memory_space=pl.ANY),
        ],
        out_specs=pl.BlockSpec(memory_space=pl.ANY),
        scratch_shapes=[
            pltpu.VMEM((D, 3 * D), jnp.bfloat16),
            pltpu.VMEM((D, D), jnp.bfloat16),
            pltpu.VMEM((F, D), jnp.bfloat16),
            pltpu.VMEM((F, D), jnp.bfloat16),
            pltpu.VMEM((3 * D, D), jnp.bfloat16),
            pltpu.VMEM((G, GR, _QK_W), jnp.bfloat16),
            pltpu.VMEM((D, D), jnp.bfloat16),
            pltpu.VMEM((S, D), jnp.bfloat16),
            pltpu.VMEM((2 * D, S), jnp.bfloat16),
            pltpu.VMEM((G, GA, _PHI_W), jnp.float32),
            pltpu.VMEM((G, GA, _PHI_W), jnp.bfloat16),
            pltpu.SemaphoreType.DMA((6 + 2 * NB,)),
        ],
    )
    return pl.pallas_call(
        _kernel,
        grid_spec=grid_spec,
        out_shape=jax.ShapeDtypeStruct((S, D), A_x.dtype),
        compiler_params=pltpu.CompilerParams(
            dimension_semantics=("arbitrary", "arbitrary"),
            vmem_limit_bytes=100 * 1024 * 1024,
        ),
    )(A_x.reshape(S, D), wphi2, A_wqkv, A_wo, w1_t, B_w2).reshape(A_x.shape)
```
